```python
import jax
import jax.numpy as jnp

def _softmax(x, axis=-1):
    return jax.nn.softmax(x, axis=axis)
def _gelu(x):
    return jax.nn.gelu(x, approximate=True)
def _silu(x):
    return jax.nn.silu(x)
def _sigmoid(x):
    return jax.nn.sigmoid(x)
def _layernorm(x, axis=-1, eps=1e-5):
    m = jnp.mean(x, axis=axis, keepdims=True)
    v = jnp.var(x, axis=axis, keepdims=True)
    return (x - m) / jnp.sqrt(v + eps)
def _scatter_add(tgt, idx, src, axis=0):
    return tgt.at[idx].add(src)
def _segment_sum(src, seg, n):
    return jax.ops.segment_sum(src, seg, n)
class _Rng:
    def __init__(self, key):
        self._k = key
    def _next(self):
        self._k, sub = jax.random.split(self._k)
        return sub
    def normal(self, shape):
        return jax.random.normal(self._next(), shape, dtype=jnp.bfloat16)
    def randint(self, lo, hi, shape):
        return jax.random.randint(self._next(), shape, lo, hi, dtype=jnp.int32)
    def uniform(self, shape, lo=0.0, hi=1.0):
        return jax.random.uniform(self._next(), shape, jnp.bfloat16, lo, hi)
    def permutation(self, n):
        return jax.random.permutation(self._next(), n)


kernel_name = 'recurrent_scan__sliding_block_cached__glu_gated_swiglu__decode'

def setup_inputs():
    _rng = _Rng(jax.random.key(int.from_bytes(__import__("os").urandom(4), "little")))
    _w = (lambda a: (lambda t: t.astype(jnp.bfloat16) if jnp.issubdtype(t.dtype, jnp.floating) else t)(jnp.asarray(a)))
    def _A_setup():
        B, Sq, D = 1, 1, 640
        Hq, Hkv, Sk, Dh = 32, 32, 32768, 192
        assert Hq % Hkv == 0, (Hq, Hkv)
        return {
            "x": _w((lambda *s: _rng.normal(s) * 0.05)(B, Sq, D)),
            "k_cache": _w((lambda *s: _rng.normal(s) * 0.05)(B, Hkv, Sk, Dh)),
            "v_cache": _w((lambda *s: _rng.normal(s) * 0.05)(B, Hkv, Sk, Dh)),
            "wq": _w((lambda *s: _rng.normal(s) * 0.05)(D, Hq * Dh) * (D ** -0.5)),
            "wo": _w((lambda *s: _rng.normal(s) * 0.05)(Hq * Dh, D) * ((Hq * Dh) ** -0.5)),
        }
    _A_in = _A_setup()

    def _B_setup():
        B, S, D, F = 1, 1, 640, 1536
        return {
            "x": _w((lambda *s: _rng.normal(s) * 0.05)(B, S, D)),
            "w1": _w((lambda *s: _rng.normal(s) * 0.05)(D, F) * (2.0 / D) ** 0.5),
            "w3": _w((lambda *s: _rng.normal(s) * 0.05)(D, F) * (2.0 / D) ** 0.5),
            "w2": _w((lambda *s: _rng.normal(s) * 0.05)(F, D) * (2.0 / F) ** 0.5),
        }
    _B_in = _B_setup()

    return {
        "A_x": _A_in["x"],
        "A_k_cache": _A_in["k_cache"],
        "A_v_cache": _A_in["v_cache"],
        "A_wq": _A_in["wq"],
        "A_wo": _A_in["wo"],
        "B_x": _B_in["x"],
        "B_w1": _B_in["w1"],
        "B_w3": _B_in["w3"],
        "B_w2": _B_in["w2"],
    }

def reference(A_x, A_k_cache, A_v_cache, A_wq, A_wo, B_x, B_w1, B_w3, B_w2):
    def _A_ref(x, k_cache, v_cache, wq, wo):
        B, Sq, D = x.shape
        Hq, Dh = 32, 192
        Hkv, Sk = k_cache.shape[1], k_cache.shape[2]
        W = min(4096, max(256, Sk // 4))
        rep = Hq // Hkv
        q = (lambda x, *d: x.transpose(*d))((x @ wq).reshape(B, Sq, Hq, Dh), 0, 2, 1, 3)
        k = jnp.repeat(k_cache[:, :, Sk - W:, :], rep, axis=1)
        v = jnp.repeat(v_cache[:, :, Sk - W:, :], rep, axis=1)
        scores = jnp.einsum("bhqd,bhkd->bhqk", q, k) * (Dh ** -0.5)
        p = _softmax(scores, axis=-1)
        o = jnp.einsum("bhqk,bhkd->bhqd", p, v)
        return (lambda x, *d: x.transpose(*d))(o, 0, 2, 1, 3).reshape(B, Sq, Hq * Dh) @ wo

    def _B_ref(x, w1, w3, w2):
        gate = jnp.einsum("bsd,df->bsf", x, w1)
        up = jnp.einsum("bsd,df->bsf", x, w3)
        h = _silu(gate) * up
        out = jnp.einsum("bsf,fd->bsd", h, w2)
        return out

    x = A_x
    xn = _layernorm(x, axis=-1)
    s = _A_ref(xn, A_k_cache, A_v_cache, A_wq, A_wo)
    g = _silu(_B_ref(xn, B_w1, B_w3, B_w2))
    return x + s * g
```

```python
import functools

import jax
import jax.numpy as jnp
from jax import lax
import jax.experimental.pallas as pl
import jax.experimental.pallas.tpu as pltpu

_HQ, _DH = 32, 192
_PAIR = 2 * _DH
_M = 8
_NKV = 3
_EPS = 1e-5


def _kernel(x_hbm, k_hbm, v_hbm, wq_hbm, wo_hbm, w1_hbm, w3_hbm, w2_hbm, out_hbm,
            x_buf, wq_buf, wo_buf, w1_buf, w3_buf, w2_buf, k_buf, v_buf,
            q_scr, o_scr, out_buf, w_sem, wo_sem, k_sem, v_sem,
            *, window, wo_chunks):
    d = x_hbm.shape[-1]
    sk = k_hbm.shape[-1]
    n_pairs = k_hbm.shape[0] // _PAIR
    f32, bf16 = jnp.float32, jnp.bfloat16

    def kv_copy(hbm, buf, sem, j, slot):
        rows = pl.ds(pl.multiple_of(j * _PAIR, _PAIR), _PAIR)
        return pltpu.make_async_copy(
            hbm.at[rows, pl.ds(sk - window, window)], buf.at[slot], sem.at[slot])

    def wo_copy(c):
        start, size = wo_chunks[c]
        return pltpu.make_async_copy(
            wo_hbm.at[pl.ds(start, size)], wo_buf.at[pl.ds(start, size)], wo_sem.at[c])

    x_cp = pltpu.make_async_copy(x_hbm, x_buf, w_sem.at[0])
    wq_cp = pltpu.make_async_copy(wq_hbm, wq_buf, w_sem.at[1])
    w1_cp = pltpu.make_async_copy(w1_hbm, w1_buf, w_sem.at[2])
    w3_cp = pltpu.make_async_copy(w3_hbm, w3_buf, w_sem.at[3])
    w2_cp = pltpu.make_async_copy(w2_hbm, w2_buf, w_sem.at[4])
    out_cp = pltpu.make_async_copy(out_buf, out_hbm, w_sem.at[5])

    wq_cp.start()
    x_cp.start()
    w1_cp.start()
    w3_cp.start()
    w2_cp.start()
    kv_copy(k_hbm, k_buf, k_sem, 0, 0).start()
    kv_copy(v_hbm, v_buf, v_sem, 0, 0).start()

    x_cp.wait()
    x = x_buf[0].astype(f32)
    mean = jnp.mean(x, axis=-1, keepdims=True)
    xc = x - mean
    var = jnp.mean(xc * xc, axis=-1, keepdims=True)
    xn = (xc / jnp.sqrt(var + _EPS)).astype(bf16)
    xn = jnp.broadcast_to(xn, (_M, d))

    wq_cp.wait()
    for j in range(1, _NKV):
        kv_copy(k_hbm, k_buf, k_sem, j, j).start()
        kv_copy(v_hbm, v_buf, v_sem, j, j).start()
    q_scr[...] = jnp.dot(xn, wq_buf[...], preferred_element_type=f32)

    w1_cp.wait()
    gate = jnp.dot(xn, w1_buf[...], preferred_element_type=f32)
    w3_cp.wait()
    up = jnp.dot(xn, w3_buf[...], preferred_element_type=f32)
    hid = (gate * jax.nn.sigmoid(gate) * up).astype(bf16)
    w2_cp.wait()
    ffn = jnp.dot(hid, w2_buf[...], preferred_element_type=f32)
    g = (ffn * jax.nn.sigmoid(ffn))[0:1]

    row = lax.broadcasted_iota(jnp.int32, (_M, _PAIR), 0)
    lane = lax.broadcasted_iota(jnp.int32, (_M, _PAIR), 1)
    own = row == (lane >= _DH).astype(jnp.int32)
    scale = _DH ** -0.5

    def pair_step(j, carry):
        slot = lax.rem(j, _NKV)
        cols = pl.ds(pl.multiple_of(j * _PAIR, 128), _PAIR)
        q2 = jnp.where(own, q_scr[:, cols], 0.0).astype(bf16)
        kv_copy(k_hbm, k_buf, k_sem, j, slot).wait()
        s = jnp.dot(q2, k_buf[slot], preferred_element_type=f32) * scale

        @pl.when(j + _NKV < n_pairs)
        def _():
            kv_copy(k_hbm, k_buf, k_sem, j + _NKV, slot).start()

        m = jnp.max(s, axis=-1, keepdims=True)
        p = jnp.exp(s - m)
        l = jnp.sum(p, axis=-1, keepdims=True)
        kv_copy(v_hbm, v_buf, v_sem, j, slot).wait()
        o2 = lax.dot_general(p.astype(bf16), v_buf[slot], (((1,), (1,)), ((), ())),
                             preferred_element_type=f32)

        @pl.when(j + _NKV < n_pairs)
        def _():
            kv_copy(v_hbm, v_buf, v_sem, j + _NKV, slot).start()

        @pl.when(j + _NKV == n_pairs)
        def _():
            for c in range(len(wo_chunks)):
                wo_copy(c).start()

        o2 = jnp.where(own, o2 / l, 0.0)
        o_scr[:, cols] = jnp.broadcast_to(jnp.sum(o2, axis=0, keepdims=True), (_M, _PAIR))
        return carry

    lax.fori_loop(0, n_pairs, pair_step, 0)

    acc = jnp.zeros((_M, d), f32)
    for c, (start, size) in enumerate(wo_chunks):
        wo_copy(c).wait()
        acc += jnp.dot(o_scr[:, pl.ds(start, size)].astype(bf16),
                       wo_buf[pl.ds(start, size), :], preferred_element_type=f32)
    out_buf[0] = (x + acc[0:1] * g).astype(out_buf.dtype)
    out_cp.start()
    out_cp.wait()


@jax.jit
def pallas_recurrent_scan__sliding_block_cached__glu_gated_swiglu__decode_kernel(
    A_x: jax.Array,
    A_k_cache: jax.Array,
    A_v_cache: jax.Array,
    A_wq: jax.Array,
    A_wo: jax.Array,
    B_x: jax.Array,
    B_w1: jax.Array,
    B_w3: jax.Array,
    B_w2: jax.Array,
):
    del B_x
    _, _, d = A_x.shape
    _, hkv, sk, dh = A_k_cache.shape
    assert A_x.shape[:2] == (1, 1) and (hkv, dh) == (_HQ, _DH)
    window = min(4096, max(256, sk // 4))
    hd = hkv * dh
    f = B_w1.shape[1]
    dt = A_x.dtype

    kt = jnp.transpose(A_k_cache, (0, 1, 3, 2)).reshape(hd, sk)
    vt = jnp.transpose(A_v_cache, (0, 1, 3, 2)).reshape(hd, sk)

    wo_chunks = ((0, 2048), (2048, 2048), (4096, 1024), (5120, 512), (5632, 384), (6016, 128))
    hbm = pl.BlockSpec(memory_space=pltpu.HBM)
    return pl.pallas_call(
        functools.partial(_kernel, window=window, wo_chunks=wo_chunks),
        out_shape=jax.ShapeDtypeStruct(A_x.shape, dt),
        in_specs=[hbm] * 8,
        out_specs=hbm,
        scratch_shapes=[
            pltpu.VMEM(A_x.shape, dt),
            pltpu.VMEM((d, hd), dt),
            pltpu.VMEM((hd, d), dt),
            pltpu.VMEM((d, f), dt),
            pltpu.VMEM((d, f), dt),
            pltpu.VMEM((f, d), dt),
            pltpu.VMEM((_NKV, _PAIR, window), dt),
            pltpu.VMEM((_NKV, _PAIR, window), dt),
            pltpu.VMEM((_M, hd), jnp.float32),
            pltpu.VMEM((_M, hd), jnp.float32),
            pltpu.VMEM(A_x.shape, dt),
            pltpu.SemaphoreType.DMA((6,)),
            pltpu.SemaphoreType.DMA((len(wo_chunks),)),
            pltpu.SemaphoreType.DMA((_NKV,)),
            pltpu.SemaphoreType.DMA((_NKV,)),
        ],
        compiler_params=pltpu.CompilerParams(vmem_limit_bytes=100 * 1024 * 1024),
    )(A_x, kt, vt, A_wq, A_wo, B_w1, B_w3, B_w2)
```

```python
import functools
import jax
import jax.numpy as jnp
from jax import lax
import jax.experimental.pallas as pl
import jax.experimental.pallas.tpu as pltpu

_HQ, _DH = 32, 192
_PAIR = 2 * _DH
_M = 8
_EPS = 1e-5
_T = 128


def _kernel(x_hbm, k_hbm, v_hbm, wq_hbm, wo_hbm, w1_hbm, w3_hbm, w2_hbm, out_hbm,
            x_buf, wq_buf, wo_buf, w1_buf, w3_buf, w2_buf, kv_buf,
            o_scr, out_buf, io_sem, wq_sem, w13_sem, w2_sem, wo_sem, kv_sem,
            *, window, look, wo_slabs, wrows, kvcols, roword):
    d = x_hbm.shape[-1]
    sk = k_hbm.shape[-1]
    hd = k_hbm.shape[0]
    f = w1_hbm.shape[1]
    n_pairs = hd // _PAIR
    f32, bf16 = jnp.float32, jnp.bfloat16

    def start_pieces(pieces):
        for i, (src, dst, sem) in enumerate(pieces):
            pltpu.make_async_copy(src, dst, sem).start(priority=i % 2)

    def wait_all(dst, sem):
        pltpu.make_async_copy(dst, dst, sem).wait()

    def w_pieces(hbm, buf, sem, r0, nr, pr, pc):
        return [(hbm.at[pl.ds(r, pr), pl.ds(c, pc)], buf.at[pl.ds(r, pr), pl.ds(c, pc)], sem)
                for r in range(r0, r0 + nr, pr) for c in range(0, hbm.shape[1], pc)]

    def wq_slab(i):
        return (lambda: start_pieces(w_pieces(wq_hbm, wq_buf, wq_sem.at[i], i * _T, _T, 8, 2048)),
                lambda: wait_all(wq_buf.at[pl.ds(i * _T, _T)], wq_sem.at[i]))

    def w13_slab(i):
        def start():
            start_pieces(w_pieces(w1_hbm, w1_buf, w13_sem.at[0, i], i * _T, _T, 8, f))
            start_pieces(w_pieces(w3_hbm, w3_buf, w13_sem.at[1, i], i * _T, _T, 8, f))
        def wait():
            wait_all(w1_buf.at[pl.ds(i * _T, _T)], w13_sem.at[0, i])
            wait_all(w3_buf.at[pl.ds(i * _T, _T)], w13_sem.at[1, i])
        return start, wait

    def w2_slab(i):
        return (lambda: start_pieces(w_pieces(w2_hbm, w2_buf, w2_sem.at[i], i * 512, 512, wrows, d)),
                lambda: wait_all(w2_buf.at[pl.ds(i * 512, 512)], w2_sem.at[i]))

    def wo_slab(i):
        r0, nr = wo_slabs[i]
        return (lambda: start_pieces(w_pieces(wo_hbm, wo_buf, wo_sem.at[i], r0, nr, wrows, d)),
                lambda: wait_all(wo_buf.at[pl.ds(r0, nr)], wo_sem.at[i]))

    def kv_start(j, t):
        hbm = k_hbm if t < 3 else v_hbm
        r0 = j * _PAIR + (t % 3) * _T
        if not isinstance(r0, int):
            r0 = pl.multiple_of(r0, _T)
        start_pieces([(hbm.at[pl.ds(r0 + r, 8), pl.ds(sk - window + c, kvcols)],
                       kv_buf.at[t, pl.ds(r, 8), pl.ds(c, kvcols)], kv_sem.at[t])
                      for r in roword for c in range(0, window, kvcols)])

    def kv_wait(t):
        wait_all(kv_buf.at[t], kv_sem.at[t])

    head = [wq_slab(i) for i in range(d // _T)] + [w13_slab(i) for i in range(d // _T)] \
        + [w2_slab(i) for i in range(f // 512)]
    tail = [wo_slab(i) for i in range(len(wo_slabs))]
    n_head = len(head)

    def start_global(i):
        if i < n_head:
            head[i][0]()
        else:
            kv_start(0, i - n_head)

    x_cp = pltpu.make_async_copy(x_hbm, x_buf, io_sem.at[0])
    out_cp = pltpu.make_async_copy(out_buf, out_hbm, io_sem.at[1])
    x_cp.start()
    for i in range(look):
        start_global(i)

    x_cp.wait()
    x = x_buf[0].astype(f32)
    mean = jnp.mean(x, axis=-1, keepdims=True)
    xc = x - mean
    var = jnp.mean(xc * xc, axis=-1, keepdims=True)
    xn = (xc / jnp.sqrt(var + _EPS)).astype(bf16)
    xn = jnp.broadcast_to(xn, (_M, d))

    step = 0
    q = jnp.zeros((_M, hd), f32)
    for i in range(d // _T):
        start_global(step + look)
        head[step][1]()
        q += jnp.dot(xn[:, i * _T:(i + 1) * _T], wq_buf[pl.ds(i * _T, _T), :], preferred_element_type=f32)
        step += 1
    o_scr[...] = q
    gate = jnp.zeros((_M, f), f32)
    up = jnp.zeros((_M, f), f32)
    for i in range(d // _T):
        start_global(step + look)
        head[step][1]()
        xi = xn[:, i * _T:(i + 1) * _T]
        gate += jnp.dot(xi, w1_buf[pl.ds(i * _T, _T), :], preferred_element_type=f32)
        up += jnp.dot(xi, w3_buf[pl.ds(i * _T, _T), :], preferred_element_type=f32)
        step += 1
    hid = (gate * jax.nn.sigmoid(gate) * up).astype(bf16)
    ffn = jnp.zeros((_M, d), f32)
    for i in range(f // 512):
        start_global(step + look)
        head[step][1]()
        ffn += jnp.dot(hid[:, i * 512:(i + 1) * 512], w2_buf[pl.ds(i * 512, 512), :], preferred_element_type=f32)
        step += 1
    g = (ffn * jax.nn.sigmoid(ffn))[0:1]

    row = lax.broadcasted_iota(jnp.int32, (_M, _PAIR), 0)
    lane = lax.broadcasted_iota(jnp.int32, (_M, _PAIR), 1)
    own = row == (lane >= _DH).astype(jnp.int32)
    scale = _DH ** -0.5

    def pair_step(j, last):
        def prefetch(t):
            nt = t + look
            if nt < 6:
                kv_start(j, nt)
            elif not last:
                kv_start(j + 1, nt - 6)
            elif nt - 6 < len(tail):
                tail[nt - 6][0]()

        c0 = j * _PAIR
        cols = pl.ds(c0 if last else pl.multiple_of(c0, 128), _PAIR)
        q2 = jnp.where(own, o_scr[:, cols], 0.0).astype(bf16)
        s = jnp.zeros((_M, window), f32)
        for t in range(3):
            prefetch(t)
            kv_wait(t)
            s += jnp.dot(q2[:, t * _T:(t + 1) * _T], kv_buf[t], preferred_element_type=f32)
        s = s * scale
        m = jnp.max(s, axis=-1, keepdims=True)
        p = jnp.exp(s - m)
        l = jnp.sum(p, axis=-1, keepdims=True)
        p = p.astype(bf16)
        o2 = []
        for t in range(3, 6):
            prefetch(t)
            kv_wait(t)
            o2.append(lax.dot_general(p, kv_buf[t], (((1,), (1,)), ((), ())), preferred_element_type=f32))
        o2 = jnp.where(own, jnp.concatenate(o2, axis=1) / l, 0.0)
        o_scr[:, cols] = jnp.broadcast_to(jnp.sum(o2, axis=0, keepdims=True), (_M, _PAIR))

    def body(j, c):
        pair_step(j, False)
        return c
    lax.fori_loop(0, n_pairs - 1, body, 0)
    pair_step(n_pairs - 1, True)

    acc = jnp.zeros((_M, d), f32)
    for i, (r0, nr) in enumerate(wo_slabs):
        if i + look < len(tail):
            tail[i + look][0]()
        tail[i][1]()
        acc += jnp.dot(o_scr[:, pl.ds(r0, nr)].astype(bf16), wo_buf[pl.ds(r0, nr), :], preferred_element_type=f32)
    out_buf[0] = (x + acc[0:1] * g).astype(out_buf.dtype)
    out_cp.start()
    out_cp.wait()


def make(look=4, wrows=16, kvcols=2048, roword=None, wo_slabs=None, nochk=True):
    if wo_slabs is None:
        wo_slabs = tuple((i * 512, 512) for i in range(11)) + ((5632, 384), (6016, 128))
    if roword is None:
        roword = tuple(range(0, _T, 8))
    def fn(A_x, A_k_cache, A_v_cache, A_wq, A_wo, B_x, B_w1, B_w3, B_w2):
        _, _, d = A_x.shape
        _, hkv, sk, dh = A_k_cache.shape
        window = min(4096, max(256, sk // 4))
        hd = hkv * dh
        f = B_w1.shape[1]
        dt = A_x.dtype
        kt = jnp.transpose(A_k_cache, (0, 1, 3, 2)).reshape(hd, sk)
        vt = jnp.transpose(A_v_cache, (0, 1, 3, 2)).reshape(hd, sk)
        hbm = pl.BlockSpec(memory_space=pltpu.HBM)
        return pl.pallas_call(
            functools.partial(_kernel, window=window, look=look, wo_slabs=wo_slabs, wrows=wrows, kvcols=kvcols, roword=roword),
            out_shape=jax.ShapeDtypeStruct(A_x.shape, dt),
            in_specs=[hbm] * 8,
            out_specs=hbm,
            scratch_shapes=[
                pltpu.VMEM(A_x.shape, dt),
                pltpu.VMEM((d, hd), dt),
                pltpu.VMEM((hd, d), dt),
                pltpu.VMEM((d, f), dt),
                pltpu.VMEM((d, f), dt),
                pltpu.VMEM((f, d), dt),
                pltpu.VMEM((6, _T, window), dt),
                pltpu.VMEM((_M, hd), jnp.float32),
                pltpu.VMEM(A_x.shape, dt),
                pltpu.SemaphoreType.DMA((2,)),
                pltpu.SemaphoreType.DMA((d // _T,)),
                pltpu.SemaphoreType.DMA((2, d // _T)),
                pltpu.SemaphoreType.DMA((f // 512,)),
                pltpu.SemaphoreType.DMA((len(wo_slabs),)),
                pltpu.SemaphoreType.DMA((6,)),
            ],
            compiler_params=pltpu.CompilerParams(vmem_limit_bytes=100 * 1024 * 1024, disable_bounds_checks=nochk),
        )(A_x, kt, vt, A_wq, A_wo, B_w1, B_w3, B_w2)
    return fn

pallas_recurrent_scan__sliding_block_cached__glu_gated_swiglu__decode_kernel = jax.jit(make(nochk=False))
```

```python
import functools

import jax
import jax.numpy as jnp
from jax import lax
import jax.experimental.pallas as pl
import jax.experimental.pallas.tpu as pltpu

_HQ, _DH = 32, 192
_PAIR = 2 * _DH
_T = 128
_SLOTS = 6
_LOOK = 4
_M = 8
_EPS = 1e-5


def _loop(lo, hi, body):
    def step(i, carry):
        body(i)
        return carry
    lax.fori_loop(lo, hi, step, 0)


def _div3(n):
    return (n * 43691) >> 17


def _kernel(x_hbm, k_hbm, v_hbm, wq_hbm, wo_hbm, w1_hbm, w3_hbm, w2_hbm, out_hbm,
            x_buf, wq_buf, wo_buf, w1_buf, w3_buf, w2_buf, kv_buf,
            qo_scr, h_scr, out_buf, sem, *, window):
    d = x_hbm.shape[-1]
    hd, sk = k_hbm.shape
    f = w1_hbm.shape[1]
    n_pairs = hd // _PAIR
    n_groups = hd // (4 * _T)
    f32, bf16 = jnp.float32, jnp.bfloat16

    def start(src, dst, s, thread):
        pltpu.make_async_copy(src, dst, s).start(priority=thread)

    def wait_for(dst, s):
        pltpu.make_async_copy(dst, dst, s).wait()

    def issue_wq(s):
        def phase(p):
            def pair(k):
                for t in range(2):
                    b = 16 * k + 2 * p + t
                    r = _div3(b)
                    idx = (pl.ds(pl.multiple_of(r * 8, 8), 8),
                           pl.ds(pl.multiple_of((b - 3 * r) * 2048, 2048), 2048))
                    start(wq_hbm.at[idx], wq_buf.at[idx], s, t)
            _loop(0, 15, pair)
        _loop(0, 8, phase)

    def issue_w13(hbm, buf, s, lo, hi):
        def pair(i):
            p = (i & 3) * 10 + (i >> 2)
            for t in range(2):
                rows = pl.ds(pl.multiple_of(p * 16 + t * 8, 8), 8)
                start(hbm.at[rows], buf.at[rows], s, t)
        _loop(lo, hi, pair)

    def group_chunk(g):
        blk = _div3(g)
        return blk * 12 + (g - 3 * blk)

    def issue_group(hbm, buf, s, g):
        c0 = group_chunk(g)
        def quarter(i):
            for k in range(4):
                for t in range(2):
                    r = (c0 + 3 * k) * _T + i * 32 + t * 16
                    rows = pl.ds(pl.multiple_of(r, 16), 16)
                    start(hbm.at[rows], buf.at[rows], s, t)
        _loop(0, 4, quarter)

    def chunk_rows(c):
        return pl.ds(pl.multiple_of(c * _T, _T), _T)

    def project(lhs_scr, buf, chunks, acc):
        for c in chunks:
            acc += jnp.dot(lhs_scr[:, chunk_rows(c)].astype(bf16), buf[chunk_rows(c), :],
                           preferred_element_type=f32)
        return acc

    def issue_kv(j, t):
        hbm = k_hbm if t < 3 else v_hbm
        r0 = j * _PAIR + (t % 3) * _T
        half = window // 2
        def tile_row(i):
            r = ((i & 7) * 2 + (i >> 3)) * 8
            for c in range(2):
                start(hbm.at[pl.ds(pl.multiple_of(r0 + r, 8), 8), pl.ds(sk - window + c * half, half)],
                      kv_buf.at[t, pl.ds(pl.multiple_of(r, 8), 8), pl.ds(c * half, half)],
                      sem.at[t], c)
        _loop(0, _T // 8, tile_row)

    x_cp = pltpu.make_async_copy(x_hbm, x_buf, sem.at[0])
    x_cp.start()
    issue_wq(sem.at[3])
    x_cp.wait()
    x = x_buf[0].astype(f32)
    xc = x - jnp.mean(x, axis=-1, keepdims=True)
    var = jnp.mean(xc * xc, axis=-1, keepdims=True)
    xn = jnp.broadcast_to((xc / jnp.sqrt(var + _EPS)).astype(bf16), (_M, d))
    issue_w13(w1_hbm, w1_buf, sem.at[4], 0, 40)

    wait_for(wq_buf, sem.at[3])

    def q_chunk(c):
        cols = pl.ds(pl.multiple_of(c * 1024, 1024), 1024)
        qo_scr[:, cols] = jnp.dot(xn, wq_buf[:, cols], preferred_element_type=f32)

        @pl.when(c < 5)
        def _():
            issue_w13(w3_hbm, w3_buf, sem.at[5], c * 8, c * 8 + 8)
    _loop(0, hd // 1024, q_chunk)

    _loop(0, f // (4 * _T), lambda g: issue_group(w2_hbm, w2_buf, sem.at[3], g))
    wait_for(w1_buf, sem.at[4])
    wait_for(w3_buf, sem.at[5])

    def h_chunk(c):
        cols = pl.ds(pl.multiple_of(c * 512, 512), 512)
        gate = jnp.dot(xn, w1_buf[:, cols], preferred_element_type=f32)
        up = jnp.dot(xn, w3_buf[:, cols], preferred_element_type=f32)
        h_scr[:, cols] = gate * jax.nn.sigmoid(gate) * up
        for t in range(3):
            pl.when(c == t)(functools.partial(issue_kv, 0, t))
    _loop(0, f // 512, h_chunk)

    wait_for(w2_buf, sem.at[3])
    issue_kv(0, 3)
    ffn = lax.fori_loop(
        0, f // 512,
        lambda g, acc: project(h_scr, w2_buf, [4 * g + k for k in range(4)], acc),
        jnp.zeros((_M, d), f32))
    gate_out = (ffn * jax.nn.sigmoid(ffn))[0:1]

    row = lax.broadcasted_iota(jnp.int32, (_M, _PAIR), 0)
    lane = lax.broadcasted_iota(jnp.int32, (_M, _PAIR), 1)
    own = row == (lane >= _DH).astype(jnp.int32)

    def pair_step(j):
        def advance(t):
            nt = t + _LOOK
            if nt < _SLOTS:
                issue_kv(j, nt)
            else:
                nt -= _SLOTS
                pl.when(j + 1 < n_pairs)(functools.partial(issue_kv, j + 1, nt))
                pl.when(j + 1 == n_pairs)(
                    functools.partial(issue_group, wo_hbm, wo_buf, sem.at[nt], nt))
            wait_for(kv_buf.at[t], sem.at[t])

        cols = pl.ds(pl.multiple_of(j * _PAIR, 128), _PAIR)
        q2 = jnp.where(own, qo_scr[:, cols], 0.0).astype(bf16)
        s = jnp.zeros((_M, window), f32)
        for t in range(3):
            advance(t)
            s += jnp.dot(q2[:, t * _T:(t + 1) * _T], kv_buf[t], preferred_element_type=f32)
        s = s * _DH ** -0.5
        p = jnp.exp(s - jnp.max(s, axis=-1, keepdims=True))
        denom = jnp.sum(p, axis=-1, keepdims=True)
        p = p.astype(bf16)
        o2 = []
        for t in range(3, 6):
            advance(t)
            o2.append(lax.dot_general(p, kv_buf[t], (((1,), (1,)), ((), ())),
                                      preferred_element_type=f32))
        o2 = jnp.where(own, jnp.concatenate(o2, axis=1) / denom, 0.0)
        qo_scr[:, cols] = jnp.broadcast_to(jnp.sum(o2, axis=0, keepdims=True), (_M, _PAIR))
    _loop(0, n_pairs, pair_step)

    def ring(g):
        return sem.at[jnp.where(g >= _SLOTS, g - _SLOTS, g)]

    def wo_step(g, acc):
        pl.when(g + _LOOK < n_groups)(
            lambda: issue_group(wo_hbm, wo_buf, ring(g + _LOOK), g + _LOOK))
        c0 = group_chunk(g)
        chunks = [c0 + 3 * k for k in range(4)]
        for c in chunks:
            wait_for(wo_buf.at[chunk_rows(c)], ring(g))
        return project(qo_scr, wo_buf, chunks, acc)
    acc = lax.fori_loop(0, n_groups, wo_step, jnp.zeros((_M, d), f32))

    out_buf[0] = (x + acc[0:1] * gate_out).astype(out_buf.dtype)
    out_cp = pltpu.make_async_copy(out_buf, out_hbm, sem.at[0])
    out_cp.start()
    out_cp.wait()


@jax.jit
def pallas_recurrent_scan__sliding_block_cached__glu_gated_swiglu__decode_kernel(
    A_x: jax.Array,
    A_k_cache: jax.Array,
    A_v_cache: jax.Array,
    A_wq: jax.Array,
    A_wo: jax.Array,
    B_x: jax.Array,
    B_w1: jax.Array,
    B_w3: jax.Array,
    B_w2: jax.Array,
):
    del B_x
    d = A_x.shape[-1]
    _, hkv, sk, dh = A_k_cache.shape
    hd = hkv * dh
    f = B_w1.shape[1]
    window = min(4096, max(256, sk // 4))
    assert A_x.shape == (1, 1, 640) and (hkv, dh, f) == (_HQ, _DH, 1536)
    assert window % 256 == 0 and sk % 128 == 0
    dt = A_x.dtype

    kt = jnp.transpose(A_k_cache, (0, 1, 3, 2)).reshape(hd, sk)
    vt = jnp.transpose(A_v_cache, (0, 1, 3, 2)).reshape(hd, sk)

    hbm = pl.BlockSpec(memory_space=pltpu.HBM)
    return pl.pallas_call(
        functools.partial(_kernel, window=window),
        out_shape=jax.ShapeDtypeStruct(A_x.shape, dt),
        in_specs=[hbm] * 8,
        out_specs=hbm,
        scratch_shapes=[
            pltpu.VMEM(A_x.shape, dt),
            pltpu.VMEM((d, hd), dt),
            pltpu.VMEM((hd, d), dt),
            pltpu.VMEM((d, f), dt),
            pltpu.VMEM((d, f), dt),
            pltpu.VMEM((f, d), dt),
            pltpu.VMEM((_SLOTS, _T, window), dt),
            pltpu.VMEM((_M, hd), jnp.float32),
            pltpu.VMEM((_M, f), jnp.float32),
            pltpu.VMEM(A_x.shape, dt),
            pltpu.SemaphoreType.DMA((_SLOTS,)),
        ],
        compiler_params=pltpu.CompilerParams(vmem_limit_bytes=64 * 1024 * 1024),
    )(A_x, kt, vt, A_wq, A_wo, B_w1, B_w3, B_w2)
```
